```python
import os as _os
_os.environ.setdefault("JAX_PLATFORMS", "cpu")
import jax
import jax.numpy as jnp

def _softmax(x, axis=-1):
    return jax.nn.softmax(x, axis=axis)
def _gelu(x):
    return jax.nn.gelu(x, approximate=True)
def _silu(x):
    return jax.nn.silu(x)
def _sigmoid(x):
    return jax.nn.sigmoid(x)
def _layernorm(x, axis=-1, eps=1e-5):
    m = jnp.mean(x, axis=axis, keepdims=True)
    v = jnp.var(x, axis=axis, keepdims=True)
    return (x - m) / jnp.sqrt(v + eps)
def _scatter_add(tgt, idx, src, axis=0):
    return tgt.at[idx].add(src)
def _segment_sum(src, seg, n):
    return jax.ops.segment_sum(src, seg, n)
class _Rng:
    def __init__(self, key):
        self._k = key
    def _next(self):
        self._k, sub = jax.random.split(self._k)
        return sub
    def normal(self, shape):
        return jax.random.normal(self._next(), shape, dtype=jnp.bfloat16)
    def randint(self, lo, hi, shape):
        return jax.random.randint(self._next(), shape, lo, hi, dtype=jnp.int32)
    def uniform(self, shape, lo=0.0, hi=1.0):
        return jax.random.uniform(self._next(), shape, jnp.bfloat16, lo, hi)
    def permutation(self, n):
        return jax.random.permutation(self._next(), n)


kernel_name = 'standalone__gqa_block_cached__near_ridge'

def setup_inputs():
    _rng = _Rng(jax.random.key(int.from_bytes(__import__("os").urandom(4), "little")))
    _w = (lambda a: (lambda t: t.astype(jnp.bfloat16) if jnp.issubdtype(t.dtype, jnp.floating) else t)(jnp.asarray(a)))
    B, Sq, D = 8, 64, 512
    Hq, Hkv, Sk, Dh = 32, 8, 64, 128
    assert Hq % Hkv == 0, (Hq, Hkv)
    return {
        "x": _w((lambda *s: _rng.normal(s) * 0.8)(B, Sq, D)),
        "k_cache": _w((lambda *s: _rng.normal(s) * 0.8)(B, Hkv, Sk, Dh)),
        "v_cache": _w((lambda *s: _rng.normal(s) * 0.05)(B, Hkv, Sk, Dh)),
        "wq": _w((lambda *s: _rng.normal(s) * 0.8)(D, Hq * Dh) * (D ** -0.5)),
        "wo": _w((lambda *s: _rng.normal(s) * 0.05)(Hq * Dh, D) * ((Hq * Dh) ** -0.5)),
    }

def reference(x, k_cache, v_cache, wq, wo):
    B, Sq, D = x.shape
    Hq, Dh = 32, 128
    Hkv = k_cache.shape[1]
    rep = Hq // Hkv
    q = (lambda x, *d: x.transpose(*d))((x @ wq).reshape(B, Sq, Hq, Dh), 0, 2, 1, 3)
    k = jnp.repeat(k_cache, rep, axis=1)
    v = jnp.repeat(v_cache, rep, axis=1)
    scores = jnp.einsum("bhqd,bhkd->bhqk", q, k) * (Dh ** -0.5)
    p = _softmax(scores, axis=-1)
    o = jnp.einsum("bhqk,bhkd->bhqd", p, v)
    return (lambda x, *d: x.transpose(*d))(o, 0, 2, 1, 3).reshape(B, Sq, Hq * Dh) @ wo
```

```python
import jax
import jax.numpy as jnp
from jax import lax
import jax.experimental.pallas as pl
import jax.experimental.pallas.tpu as pltpu

_LANE = 128
_LOG2E = 1.4426950408889634
_NT = (((1,), (1,)), ((), ()))
_TN = (((0,), (0,)), ((), ()))
_NQ = 3


def _schedule(n_groups, rep, n_batch, nd):
    assert (n_groups, rep, n_batch, nd) == (8, 4, 8, 4), "the hand schedule assumes these counts"
    G = n_groups

    def wq(h0, h1, j0=0, j1=nd):
        return [("wq", h, j0, j1) for h in range(h0, h1)]

    def step_data(t):
        items = []
        if t + 1 < G:
            items += wq(rep * (t + 1), rep * (t + 2))
        if 1 <= t <= G:
            items += [("k", t - 1), ("v", t - 1)]
        if t >= 2:
            items += [("wo", t - 2, 0, nd)]
        return items

    copies = {}
    ops = []

    for j in range(nd):
        copies[f"wa{j}"] = wq(0, rep, j, j + 1)
        copies[f"x{j}"] = [("x", j)]
        copies[f"wb{j}"] = wq(rep, 2 * rep, j, j + 1)
        ops += [("W", f"wa{j}"), ("W", f"x{j}")]
        parts = 4 if j == 0 else 1
        ops += [("Q", 0, j, p, parts) for p in range(parts)]
        ops += [("W", f"wb{j}"), ("Q", 1, j, 0, 1)]

    copies.update(
        k0=[("k", 0)], h8=wq(8, 9), v0=[("v", 0)], h9=wq(9, 10), h10=wq(10, 12),
        wo0a=[("wo", 0, 0, 1)], kv1=[("k", 1), ("v", 1)], h12=wq(12, 13),
        wo0b=[("wo", 0, 1, nd)], h13=wq(13, 16),
        s3=step_data(3), s4=step_data(4), s5=step_data(5),
        s6=[it for t in range(6, G + 2) for it in step_data(t)],
    )

    steady = "O0 K0 K1 P0 V0 V1 K2 K3 O1 V2 V3 K4 K5 P1 V4 V5 K6 K7 O2 V6 V7 P2 O3 P3"
    no_qp = "K0 K1 O0 V0 V1 K2 K3 O1 V2 V3 K4 K5 O2 V4 V5 K6 K7 O3 V6 V7"
    steps = {
        1: "W:k0 K0 K1 W:h8 P0 W:v0 V0 V1 K2 K3 W:h9 P1 V2 V3 K4 K5 W:h10 P2 V4 V5 K6 K7 P3 V6 V7",
        2: "W:wo0a O0 W:kv1 K0 K1 W:h12 P0 V0 V1 K2 K3 W:wo0b O1 V2 V3 K4 K5 W:h13 P1 V4 V5 K6 K7"
           " O2 V6 V7 P2 O3 P3",
        3: "W:s3 " + steady,
        4: "W:s4 " + steady,
        5: "W:s5 " + steady,
        6: "W:s6 " + steady,
        7: no_qp,
        8: no_qp,
        9: "O0 O1 O2_0_2 O2_1_2 O3_0_2 O3_1_2",
    }
    for t in range(1, G + 2):
        for tok in steps[t].split():
            if tok.startswith("W:"):
                ops.append(("W", tok[2:]))
            elif tok[0] == "P":
                ops.append(("P", t + 1, int(tok[1:])))
            elif tok[0] in "KV":
                ops.append((tok[0], t - 1, int(tok[1:])))
            else:
                n, p, m = (tok[1:].split("_") + ["0", "1"])[:3]
                ops.append(("O", t - 2, int(n), int(p), int(m)))
    return copies, ops


def _make_kernel(B, Sq, D, Hq, Hkv, Sk, Dh, copies, ops):
    rep = Hq // Hkv
    T = B * Sq
    ND = D // _LANE
    f32, bf16 = jnp.float32, jnp.bfloat16
    exp2_scale = (Dh ** -0.5) * _LOG2E

    def kernel(x_hbm, k_hbm, v_hbm, wq_hbm, wo_hbm, o_hbm,
               x_s, k_s, v_s, wq_s, wo_s, q_s, o_s, qacc_s, acc_s, out_s, sems):
        def src_dst(item):
            kind = item[0]
            if kind == "x":
                j = item[1]
                return x_hbm.at[:, pl.ds(j * _LANE, _LANE)], x_s.at[j]
            if kind == "wq":
                h, j0, j1 = item[1:]
                rows = pl.ds(j0 * _LANE, (j1 - j0) * _LANE)
                return wq_hbm.at[rows, pl.ds(h * Dh, Dh)], wq_s.at[h, rows, :]
            if kind == "k":
                return k_hbm.at[:, item[1]], k_s.at[:, item[1]]
            if kind == "v":
                return v_hbm.at[:, item[1]], v_s.at[:, item[1]]
            g, n0, n1 = item[1:]
            cols = pl.ds(n0 * _LANE, (n1 - n0) * _LANE)
            return wo_hbm.at[pl.ds(g * rep * Dh, rep * Dh), cols], wo_s.at[g, :, cols]

        in_copies = {}
        for i, (name, items) in enumerate(copies.items()):
            in_copies[name] = [pltpu.make_async_copy(*src_dst(it), sems.at[i]) for it in items]
        out_sem = sems.at[len(copies)]
        for group in in_copies.values():
            for cp in group:
                cp.start()

        def q_proj_slab(g, j, part, parts):
            rows = pl.ds(part * (T // parts), T // parts)
            xj = x_s[j, rows, :]
            for hh in range(rep):
                h = g * rep + hh
                r = jnp.dot(xj, wq_s[h, pl.ds(j * _LANE, _LANE), :], preferred_element_type=f32)
                if j == 0:
                    qacc_s[h, rows, :] = r
                elif j < ND - 1:
                    qacc_s[h, rows, :] += r
                else:
                    q_s[g % _NQ, hh, rows, :] = (qacc_s[h, rows, :] + r).astype(bf16)

        def q_proj(g, hh):
            x = jnp.concatenate([x_s[j] for j in range(ND)], axis=1)
            q = jnp.dot(x, wq_s[g * rep + hh], preferred_element_type=f32)
            q_s[g % _NQ, hh] = q.astype(bf16)

        probs = {}

        def scores_softmax(g, b):
            rows = pl.ds(b * Sq, Sq)
            q = jnp.concatenate([q_s[g % _NQ, hh, rows, :] for hh in range(rep)], axis=0)
            s = lax.dot_general(k_s[b, g], q, _NT, preferred_element_type=f32)
            m = jnp.max(s, axis=0, keepdims=True)
            p = jnp.exp2((s - m) * exp2_scale)
            l = jnp.sum(p, axis=0, keepdims=True)
            r = pltpu.reciprocal(l, approx=True)
            r = r * (2.0 - l * r)
            probs[g, b] = (p * r).astype(bf16)

        def prob_v(g, b):
            o = lax.dot_general(probs.pop((g, b)), v_s[b, g], _TN, preferred_element_type=f32)
            o = o.astype(bf16)
            for hh in range(rep):
                o_s[g % 2, hh, pl.ds(b * Sq, Sq), :] = o[hh * Sq:(hh + 1) * Sq, :]

        out_copies = []

        def out_proj(g, n, part, parts):
            rows = pl.ds(part * (T // parts), T // parts)
            cols = pl.ds(n * _LANE, _LANE)
            o = jnp.concatenate([o_s[g % 2, hh, rows, :] for hh in range(rep)], axis=1)
            r = jnp.dot(o, wo_s[g, :, cols], preferred_element_type=f32)
            if g == 0:
                acc_s[n, rows, :] = r
            elif g < Hkv - 1:
                acc_s[n, rows, :] += r
            else:
                out_s[n, rows, :] = (acc_s[n, rows, :] + r).astype(out_s.dtype)
                cp = pltpu.make_async_copy(out_s.at[n, rows, :], o_hbm.at[rows, cols], out_sem)
                cp.start()
                out_copies.append(cp)

        for op in ops:
            kind = op[0]
            if kind == "W":
                for cp in in_copies[op[1]]:
                    cp.wait()
            elif kind == "Q":
                q_proj_slab(*op[1:])
            elif kind == "P":
                q_proj(*op[1:])
            elif kind == "K":
                scores_softmax(*op[1:])
            elif kind == "V":
                prob_v(*op[1:])
            else:
                out_proj(*op[1:])
        for cp in out_copies:
            cp.wait()

    return kernel


@jax.jit
def pallas_standalone__gqa_block_cached__near_ridge_kernel(
    x: jax.Array,
    k_cache: jax.Array,
    v_cache: jax.Array,
    wq: jax.Array,
    wo: jax.Array,
):
    B, Sq, D = x.shape
    _, Hkv, Sk, Dh = k_cache.shape
    Hq = wq.shape[1] // Dh
    rep = Hq // Hkv
    T = B * Sq
    ND = D // _LANE
    assert Dh == _LANE and D % _LANE == 0 and Hq % Hkv == 0 and wo.shape == (Hq * Dh, D)

    copies, ops = _schedule(Hkv, rep, B, ND)
    bf16, f32 = jnp.bfloat16, jnp.float32
    hbm = pl.BlockSpec(memory_space=pl.ANY)

    out = pl.pallas_call(
        _make_kernel(B, Sq, D, Hq, Hkv, Sk, Dh, copies, ops),
        in_specs=[hbm] * 5,
        out_specs=hbm,
        out_shape=jax.ShapeDtypeStruct((T, D), x.dtype),
        scratch_shapes=[
            pltpu.VMEM((ND, T, _LANE), x.dtype),
            pltpu.VMEM((B, Hkv, Sk, Dh), k_cache.dtype),
            pltpu.VMEM((B, Hkv, Sk, Dh), v_cache.dtype),
            pltpu.VMEM((Hq, D, Dh), wq.dtype),
            pltpu.VMEM((Hkv, rep * Dh, D), wo.dtype),
            pltpu.VMEM((_NQ, rep, T, Dh), bf16),
            pltpu.VMEM((2, rep, T, Dh), bf16),
            pltpu.VMEM((2 * rep, T, Dh), f32),
            pltpu.VMEM((ND, T, _LANE), f32),
            pltpu.VMEM((ND, T, _LANE), x.dtype),
            pltpu.SemaphoreType.DMA((len(copies) + 1,)),
        ],
        compiler_params=pltpu.CompilerParams(
            vmem_limit_bytes=64 * 1024 * 1024,
            disable_semaphore_checks=True,
            flags={"XLA_TPU_RESCHEDULE_DMA_DONES": True},
        ),
    )(x.reshape(T, D), k_cache, v_cache, wq, wo)
    return out.reshape(B, Sq, D)
```

```python
import jax
import jax.numpy as jnp
from jax import lax
import jax.experimental.pallas as pl
import jax.experimental.pallas.tpu as pltpu

_LANE = 128
_LOG2E = 1.4426950408889634
_NT = (((1,), (1,)), ((), ()))
_TN = (((0,), (0,)), ((), ()))
_NQ = 3


def _schedule(n_groups, rep, n_batch, nd):
    assert (n_groups, rep, n_batch, nd) == (8, 4, 8, 4), "the hand schedule assumes these counts"
    G = n_groups

    def wq(h0, h1, j0=0, j1=nd):
        return [("wq", h, j0, j1) for h in range(h0, h1)]

    def step_data(t):
        items = []
        if t + 1 < G:
            items += wq(rep * (t + 1), rep * (t + 2))
        if 1 <= t <= G:
            items += [("k", t - 1), ("v", t - 1)]
        if t >= 2:
            items += [("wo", t - 2, 0, nd)]
        return items

    copies = {}
    ops = []

    parts = 4
    for j in range(nd):
        copies[f"wa{j}"] = wq(0, rep, j, j + 1)
        ops.append(("W", f"wa{j}"))
        if j == 0:
            for p in range(parts):
                copies[f"x0p{p}"] = [("x", 0, p, parts)]
                ops += [("W", f"x0p{p}"), ("Q", 0, 0, p, parts)]
        else:
            copies[f"x{j}"] = [("x", j, 0, 1)]
            ops.append(("W", f"x{j}"))
            ops += [("Q", 0, j, p, parts) for p in range(parts)]
        copies[f"wb{j}"] = wq(rep, 2 * rep, j, j + 1)
        ops.append(("W", f"wb{j}"))
        ops += [("Q", 1, j, p, parts) for p in range(parts)]

    copies.update(
        k0=[("k", 0)], h8=wq(8, 9), v0=[("v", 0)], h9=wq(9, 10), h10=wq(10, 12),
        wo0a=[("wo", 0, 0, 1)], kv1=[("k", 1), ("v", 1)], h12=wq(12, 13),
        wo0b=[("wo", 0, 1, nd)], h13=wq(13, 16),
        s3=step_data(3), s4=step_data(4), s5=step_data(5),
        s6=[it for t in range(6, G + 2) for it in step_data(t)],
    )

    steady = "O0 K0 K1 P0 V0 V1 K2 K3 O1 V2 V3 K4 K5 P1 V4 V5 K6 K7 O2 V6 V7 P2 O3 P3"
    no_qp = "K0 K1 O0 K2 K3 V0 V1 O1 K4 K5 V2 V3 O2 K6 K7 V4 V5 O3 V6 V7"
    steps = {
        1: "W:k0 K0 K1 W:h8 P0 W:v0 V0 V1 K2 K3 W:h9 P1 V2 V3 K4 K5 W:h10 P2 V4 V5 K6 K7 P3 V6 V7",
        2: "W:wo0a O0 W:kv1 K0 K1 W:h12 P0 V0 V1 K2 K3 W:wo0b O1 V2 V3 K4 K5 W:h13 P1 V4 V5 K6 K7"
           " O2 V6 V7 P2 O3 P3",
        3: "W:s3 " + steady,
        4: "W:s4 " + steady,
        5: "W:s5 " + steady,
        6: "W:s6 " + steady,
        7: no_qp,
        8: no_qp,
        9: "O0 O1 O2_0_2 O2_1_2 O3_0_2 O3_2_4 O3_6_8 O3_7_8",
    }
    for t in range(1, G + 2):
        for tok in steps[t].split():
            if tok.startswith("W:"):
                ops.append(("W", tok[2:]))
            elif tok[0] == "P":
                ops.append(("P", t + 1, int(tok[1:])))
            elif tok[0] in "KV":
                ops.append((tok[0], t - 1, int(tok[1:])))
            else:
                n, p, m = (tok[1:].split("_") + ["0", "1"])[:3]
                ops.append(("O", t - 2, int(n), int(p), int(m)))
    return copies, ops


def _make_kernel(B, Sq, D, Hq, Hkv, Sk, Dh, copies, ops):
    rep = Hq // Hkv
    T = B * Sq
    ND = D // _LANE
    f32, bf16 = jnp.float32, jnp.bfloat16
    exp2_scale = (Dh ** -0.5) * _LOG2E

    def kernel(x_hbm, k_hbm, v_hbm, wq_hbm, wo_hbm, o_hbm,
               x_s, k_s, v_s, wq_s, wo_s, q_s, o_s, qacc_s, acc_s, out_s, sems):
        def src_dst(item):
            kind = item[0]
            if kind == "x":
                j, part, parts = item[1:]
                rows = pl.ds(part * (T // parts), T // parts)
                return x_hbm.at[rows, pl.ds(j * _LANE, _LANE)], x_s.at[j, rows, :]
            if kind == "wq":
                h, j0, j1 = item[1:]
                rows = pl.ds(j0 * _LANE, (j1 - j0) * _LANE)
                return wq_hbm.at[rows, pl.ds(h * Dh, Dh)], wq_s.at[h, rows, :]
            if kind == "k":
                return k_hbm.at[:, item[1]], k_s.at[:, item[1]]
            if kind == "v":
                return v_hbm.at[:, item[1]], v_s.at[:, item[1]]
            g, n0, n1 = item[1:]
            cols = pl.ds(n0 * _LANE, (n1 - n0) * _LANE)
            return wo_hbm.at[pl.ds(g * rep * Dh, rep * Dh), cols], wo_s.at[g, :, cols]

        in_copies = {}
        for i, (name, items) in enumerate(copies.items()):
            in_copies[name] = [pltpu.make_async_copy(*src_dst(it), sems.at[i]) for it in items]
        out_sem = sems.at[len(copies)]
        for group in in_copies.values():
            for cp in group:
                cp.start()

        def q_proj_slab(g, j, part, parts):
            rows = pl.ds(part * (T // parts), T // parts)
            xj = x_s[j, rows, :]
            for hh in range(rep):
                h = g * rep + hh
                r = jnp.dot(xj, wq_s[h, pl.ds(j * _LANE, _LANE), :], preferred_element_type=f32)
                if j == 0:
                    qacc_s[h, rows, :] = r
                elif j < ND - 1:
                    qacc_s[h, rows, :] += r
                else:
                    q_s[g % _NQ, hh, rows, :] = (qacc_s[h, rows, :] + r).astype(bf16)

        def q_proj(g, hh):
            x = jnp.concatenate([x_s[j] for j in range(ND)], axis=1)
            q = jnp.dot(x, wq_s[g * rep + hh], preferred_element_type=f32)
            q_s[g % _NQ, hh] = q.astype(bf16)

        probs = {}

        def scores_softmax(g, b):
            rows = pl.ds(b * Sq, Sq)
            q = jnp.concatenate([q_s[g % _NQ, hh, rows, :] for hh in range(rep)], axis=0)
            s = lax.dot_general(k_s[b, g], q, _NT, preferred_element_type=f32)
            m = jnp.max(s, axis=0, keepdims=True)
            p = jnp.exp2((s - m) * exp2_scale)
            l = jnp.sum(p, axis=0, keepdims=True)
            r = pltpu.reciprocal(l, approx=True)
            r = r * (2.0 - l * r)
            probs[g, b] = (p * r).astype(bf16)

        def prob_v(g, b):
            o = lax.dot_general(probs.pop((g, b)), v_s[b, g], _TN, preferred_element_type=f32)
            o = o.astype(bf16)
            for hh in range(rep):
                o_s[g % 2, hh, pl.ds(b * Sq, Sq), :] = o[hh * Sq:(hh + 1) * Sq, :]

        out_copies = []

        def out_proj(g, n, part, parts):
            rows = pl.ds(part * (T // parts), T // parts)
            cols = pl.ds(n * _LANE, _LANE)
            o = jnp.concatenate([o_s[g % 2, hh, rows, :] for hh in range(rep)], axis=1)
            r = jnp.dot(o, wo_s[g, :, cols], preferred_element_type=f32)
            if g == 0:
                acc_s[n, rows, :] = r
            elif g < Hkv - 1:
                acc_s[n, rows, :] += r
            else:
                out_s[n, rows, :] = (acc_s[n, rows, :] + r).astype(out_s.dtype)
                cp = pltpu.make_async_copy(out_s.at[n, rows, :], o_hbm.at[rows, cols], out_sem)
                cp.start()
                out_copies.append(cp)

        for op in ops:
            kind = op[0]
            if kind == "W":
                for cp in in_copies[op[1]]:
                    cp.wait()
            elif kind == "Q":
                q_proj_slab(*op[1:])
            elif kind == "P":
                q_proj(*op[1:])
            elif kind == "K":
                scores_softmax(*op[1:])
            elif kind == "V":
                prob_v(*op[1:])
            else:
                out_proj(*op[1:])
        for cp in out_copies:
            cp.wait()

    return kernel


@jax.jit
def pallas_standalone__gqa_block_cached__near_ridge_kernel(
    x: jax.Array,
    k_cache: jax.Array,
    v_cache: jax.Array,
    wq: jax.Array,
    wo: jax.Array,
):
    B, Sq, D = x.shape
    _, Hkv, Sk, Dh = k_cache.shape
    Hq = wq.shape[1] // Dh
    rep = Hq // Hkv
    T = B * Sq
    ND = D // _LANE
    assert Dh == _LANE and D % _LANE == 0 and Hq % Hkv == 0 and wo.shape == (Hq * Dh, D)

    copies, ops = _schedule(Hkv, rep, B, ND)
    bf16, f32 = jnp.bfloat16, jnp.float32
    hbm = pl.BlockSpec(memory_space=pl.ANY)

    out = pl.pallas_call(
        _make_kernel(B, Sq, D, Hq, Hkv, Sk, Dh, copies, ops),
        in_specs=[hbm] * 5,
        out_specs=hbm,
        out_shape=jax.ShapeDtypeStruct((T, D), x.dtype),
        scratch_shapes=[
            pltpu.VMEM((ND, T, _LANE), x.dtype),
            pltpu.VMEM((B, Hkv, Sk, Dh), k_cache.dtype),
            pltpu.VMEM((B, Hkv, Sk, Dh), v_cache.dtype),
            pltpu.VMEM((Hq, D, Dh), wq.dtype),
            pltpu.VMEM((Hkv, rep * Dh, D), wo.dtype),
            pltpu.VMEM((_NQ, rep, T, Dh), bf16),
            pltpu.VMEM((2, rep, T, Dh), bf16),
            pltpu.VMEM((2 * rep, T, Dh), f32),
            pltpu.VMEM((ND, T, _LANE), f32),
            pltpu.VMEM((ND, T, _LANE), x.dtype),
            pltpu.SemaphoreType.DMA((len(copies) + 1,)),
        ],
        compiler_params=pltpu.CompilerParams(
            vmem_limit_bytes=64 * 1024 * 1024,
            disable_semaphore_checks=True,
            flags={"XLA_TPU_RESCHEDULE_DMA_DONES": True},
        ),
    )(x.reshape(T, D), k_cache, v_cache, wq, wo)
    return out.reshape(B, Sq, D)
```
